```python
import jax
import jax.numpy as jnp

def _softmax(x, axis=-1):
    return jax.nn.softmax(x, axis=axis)
def _gelu(x):
    return jax.nn.gelu(x, approximate=True)
def _silu(x):
    return jax.nn.silu(x)
def _sigmoid(x):
    return jax.nn.sigmoid(x)
def _layernorm(x, axis=-1, eps=1e-5):
    m = jnp.mean(x, axis=axis, keepdims=True)
    v = jnp.var(x, axis=axis, keepdims=True)
    return (x - m) / jnp.sqrt(v + eps)
def _scatter_add(tgt, idx, src, axis=0):
    return tgt.at[idx].add(src)
def _segment_sum(src, seg, n):
    return jax.ops.segment_sum(src, seg, n)
class _Rng:
    def __init__(self, key):
        self._k = key
    def _next(self):
        self._k, sub = jax.random.split(self._k)
        return sub
    def normal(self, shape):
        return jax.random.normal(self._next(), shape, dtype=jnp.bfloat16)
    def randint(self, lo, hi, shape):
        return jax.random.randint(self._next(), shape, lo, hi, dtype=jnp.int32)
    def uniform(self, shape, lo=0.0, hi=1.0):
        return jax.random.uniform(self._next(), shape, jnp.bfloat16, lo, hi)
    def permutation(self, n):
        return jax.random.permutation(self._next(), n)


kernel_name = 'interleave_layers__sliding_local_dilated__glu_gated_geglu__prompt'

def setup_inputs():
    _rng = _Rng(jax.random.key(int.from_bytes(__import__("os").urandom(4), "little")))
    _w = (lambda a: (lambda t: t.astype(jnp.bfloat16) if jnp.issubdtype(t.dtype, jnp.floating) else t)(jnp.asarray(a)))
    def _A_setup():
        B, S, D = 1, 2048, 576
        return {
            "x": _w((lambda *s: _rng.normal(s) * 0.05)(B, S, D)),
            "wqkv": _w((lambda *s: _rng.normal(s) * 0.05)(D, 3 * D)),
            "wo": _w((lambda *s: _rng.normal(s) * 0.05)(D, D)),
        }
    _A_in = _A_setup()

    def _B_setup():
        B, S, Dm, Df = 1, 2048, 576, 4608
        return {
            "x": _w((lambda *s: _rng.normal(s) * 0.05)(B, S, Dm)),
            "w_gate": _w((lambda *s: _rng.normal(s) * 0.05)(Dm, Df) * (Dm ** -0.5)),
            "w_up": _w((lambda *s: _rng.normal(s) * 0.05)(Dm, Df) * (Dm ** -0.5)),
            "w_down": _w((lambda *s: _rng.normal(s) * 0.05)(Df, Dm) * (Df ** -0.5)),
        }
    _B_in = _B_setup()

    return {
        "A_x": _A_in["x"],
        "A_wqkv": _A_in["wqkv"],
        "A_wo": _A_in["wo"],
        "B_x": _B_in["x"],
        "B_w_gate": _B_in["w_gate"],
        "B_w_up": _B_in["w_up"],
        "B_w_down": _B_in["w_down"],
    }

def reference(A_x, A_wqkv, A_wo, B_x, B_w_gate, B_w_up, B_w_down):
    def _A_ref(x, wqkv, wo):
        B, S, D = x.shape
        H = 32; Dh = D // H
        W, dil = 8, 2
        qkv = (lambda x, *d: x.transpose(*d))((x @ wqkv).reshape(B, S, 3, H, Dh), 2, 0, 3, 1, 4)
        q, k, v = qkv[0], qkv[1], qkv[2]
        scale = Dh ** -0.5
        pos = jnp.arange(S)
        off = jnp.arange(W) * dil
        idx = pos[:, None] - off[None, :]
        mask = idx >= 0
        idx_c = jnp.where(mask, idx, 0).reshape(-1)
        kg = k[:, :, idx_c, :].reshape(B, H, S, W, Dh)
        vg = v[:, :, idx_c, :].reshape(B, H, S, W, Dh)
        logits = jnp.einsum("bhsd,bhswd->bhsw", q, kg) * scale
        logits = jnp.where(mask[None, None, :, :], logits, -1e9)
        attn = _softmax(logits, axis=-1)
        o = jnp.einsum("bhsw,bhswd->bhsd", attn, vg)
        return (lambda x, *d: x.transpose(*d))(o, 0, 2, 1, 3).reshape(B, S, D) @ wo

    def _B_ref(x, w_gate, w_up, w_down):
        g = jnp.einsum("bsd,df->bsf", x, w_gate)
        u = jnp.einsum("bsd,df->bsf", x, w_up)
        h = _gelu(g) * u
        return jnp.einsum("bsf,fd->bsd", h, w_down)

    x = A_x
    x = x + _A_ref(_layernorm(x, axis=-1), A_wqkv, A_wo)
    x = x + _B_ref(_layernorm(x, axis=-1), B_w_gate, B_w_up, B_w_down)
    x = x + _A_ref(_layernorm(x, axis=-1), A_wqkv, A_wo)
    x = x + _B_ref(_layernorm(x, axis=-1), B_w_gate, B_w_up, B_w_down)
    return x
```

```python
import numpy as np
import jax
import jax.numpy as jnp
from jax import lax
import jax.experimental.pallas as pl
import jax.experimental.pallas.tpu as pltpu

S, D, H, DH, F = 2048, 576, 32, 18, 4608
W = 8
T = 512
FC = 512
NG = 3
HG = 8
EPS = 1e-5
SCALE = DH ** -0.5
NEG = -1e9 / SCALE
NT = (((1,), (1,)), ((), ()))
U32 = jnp.uint32


def _lnT(x):
    m = jnp.mean(x, axis=0, keepdims=True)
    xc = x - m
    v = jnp.mean(xc * xc, axis=0, keepdims=True)
    return xc * lax.rsqrt(v + EPS)


def _gelu(x):
    c = 0.7978845608028654
    return 0.5 * x * (1.0 + jnp.tanh(c * (x + 0.044715 * (x * x * x))))


def _unpack(w):
    lo = pltpu.bitcast(w << 16, jnp.float32)
    hi = pltpu.bitcast(w & jnp.uint32(0xFFFF0000), jnp.float32)
    return lo, hi


def _attn_slab(qx, kx, vx, obuf, c, ocol):
    lane0 = lax.broadcasted_iota(jnp.int32, (HG, 128), 1) == 0
    for g in range(H // HG):
        acc = [None] * W
        for d in range(DH):
            r = d * H + g * HG
            q = qx[c, pl.ds(r, HG), :]
            for w in range(W):
                p = q * kx[c + 7 - w, pl.ds(r, HG), :]
                acc[w] = p if acc[w] is None else acc[w] + p
        ls = [jnp.where(lane0, NEG, acc[w]) if c < w else acc[w] for w in range(W)]
        m = ls[0]
        for w in range(1, W):
            m = jnp.maximum(m, ls[w])
        es = [jnp.exp((l - m) * SCALE) for l in ls]
        ssum = es[0]
        for w in range(1, W):
            ssum = ssum + es[w]
        inv = 1.0 / ssum
        ps = [e * inv for e in es]
        for d in range(DH):
            r = d * H + g * HG
            o = None
            for w in range(W):
                p = ps[w] * vx[c + 7 - w, pl.ds(r, HG), :]
                o = p if o is None else o + p
            obuf[pl.ds(r, HG), pl.ds(ocol, 128)] = o.astype(obuf.dtype)


def _kernel(xT_hbm, wqkv_hbm, wo_hbm, wg_hbm, wu_hbm, wdT_hbm, o_hbm,
            xin, wqkv, wo, wg, wu, wdT, wT, woP, woT, xres, qx, kx, vx, obuf, pscr, xnb, sems):
    srcs = (xT_hbm, wqkv_hbm, wo_hbm, wg_hbm, wu_hbm, wdT_hbm)
    dsts = (xin, wqkv, wo, wg, wu, wdT)
    copies = [pltpu.make_async_copy(s, d, sems.at[i]) for i, (s, d) in enumerate(zip(srcs, dsts))]
    for c in copies:
        c.start()

    copies[0].wait()
    for p0 in range(0, S, 512):
        words = pltpu.bitcast(xin[:, p0:p0 + 512].T, U32)
        for j in range(5):
            n = min(128, D - 128 * j)
            pscr[j, p0 // 2:p0 // 2 + 256, 0:n] = words[:, 128 * j:128 * j + n]
    for c in range(8):
        for j in range(5):
            n = min(128, D - 128 * j)
            wt = pscr[j, pl.ds(c, 128, stride=8), :].T
            lo, hi = _unpack(wt[0:n, :])
            xres[128 * j:128 * j + n, 128 * c:128 * c + 128] = lo
            xres[128 * j:128 * j + n, 1024 + 128 * c:1024 + 128 * c + 128] = hi

    copies[1].wait()
    for i in range(14):
        n = min(128, 3 * D - 128 * i)
        words = pltpu.bitcast(wqkv[:, 128 * i:128 * i + n].T, U32)
        for j in range(5):
            m = min(128, D - 128 * j)
            pscr[j, 64 * i:64 * i + n // 2, 0:m] = words[:, 128 * j:128 * j + m]
    for t in range(3):
        for e in range(9):
            for j in range(5):
                m = min(128, D - 128 * j)
                lo, hi = _unpack(pscr[j, pl.ds(t * 288 + e, 32, stride=9), 0:m])
                wT[t * D + 64 * e:t * D + 64 * e + 64, 128 * j:128 * j + m] = (
                    jnp.concatenate([lo, hi], axis=0).astype(jnp.bfloat16))
    copies[2].wait()
    words = pltpu.bitcast(wo[...], U32)
    for j in range(5):
        m = min(128, D - 128 * j)
        pscr[j, 0:288, 0:m] = words[:, 128 * j:128 * j + m]
    for e in range(9):
        for j in range(5):
            m = min(128, D - 128 * j)
            lo, hi = _unpack(pscr[j, pl.ds(e, 32, stride=9), 0:m])
            woP[64 * e:64 * e + 64, 128 * j:128 * j + m] = jnp.concatenate([lo, hi], axis=0).astype(jnp.bfloat16)
    woT[...] = woP[...].T

    def attn_phase():
        def par(p, _):
            c0 = pl.multiple_of(p * 1024, 1024)
            xnT = _lnT(xres[:, pl.ds(c0, 1024)]).astype(jnp.bfloat16)
            k = jnp.dot(wT[D:2 * D, :], xnT, preferred_element_type=jnp.float32)
            v = jnp.dot(wT[2 * D:3 * D, :], xnT, preferred_element_type=jnp.float32)
            q = jnp.dot(wT[0:D, :], xnT, preferred_element_type=jnp.float32)
            for c in range(8):
                kc = k[:, 128 * c:128 * c + 128]
                vc = v[:, 128 * c:128 * c + 128]
                kx[7 + c] = kc
                vx[7 + c] = vc
                if c >= 1:
                    kx[c - 1] = pltpu.roll(kc, 1, 1)
                    vx[c - 1] = pltpu.roll(vc, 1, 1)
                qx[c] = q[:, 128 * c:128 * c + 128]
            for c in range(8):
                _attn_slab(qx, kx, vx, obuf, c, 128 * c)
            y = jnp.dot(woT[...], obuf[...].astype(jnp.bfloat16), preferred_element_type=jnp.float32)
            xres[:, pl.ds(c0, 1024)] += y
            return 0
        with jax.named_scope("att"):
            lax.fori_loop(0, 2, par, 0)

    def ffn_phase():
        def tile(i, _):
            c0 = pl.multiple_of(i * T, T)
            xr = xres[:, pl.ds(c0, T)]
            xn = _lnT(xr).astype(jnp.bfloat16).T
            if NG == 1:
                acc = xr
                for c in range(F // FC):
                    g = jnp.dot(xn, wg[:, c * FC:(c + 1) * FC], preferred_element_type=jnp.float32)
                    u = jnp.dot(xn, wu[:, c * FC:(c + 1) * FC], preferred_element_type=jnp.float32)
                    h = (_gelu(g) * u).astype(jnp.bfloat16)
                    acc = acc + lax.dot_general(wdT[:, c * FC:(c + 1) * FC], h, NT, preferred_element_type=jnp.float32)
                xres[:, pl.ds(c0, T)] = acc
            else:
                xnb[...] = xn
                per = F // FC // NG

                def grp(gi, _):
                    xn = xnb[...]
                    acc = None
                    for c in range(per):
                        f0 = pl.multiple_of((gi * per + c) * FC, FC)
                        g = jnp.dot(xn, wg[:, pl.ds(f0, FC)], preferred_element_type=jnp.float32)
                        u = jnp.dot(xn, wu[:, pl.ds(f0, FC)], preferred_element_type=jnp.float32)
                        h = (_gelu(g) * u).astype(jnp.bfloat16)
                        y = lax.dot_general(wdT[:, pl.ds(f0, FC)], h, NT, preferred_element_type=jnp.float32)
                        acc = y if acc is None else acc + y
                    xres[:, pl.ds(c0, T)] += acc
                    return 0
                lax.fori_loop(0, NG, grp, 0)
            return 0
        with jax.named_scope("ffn"):
            lax.fori_loop(0, S // T, tile, 0)

    def layer(l, _):
        attn_phase()

        @pl.when(l == 0)
        def _():
            copies[3].wait(); copies[4].wait(); copies[5].wait()
        ffn_phase()
        return 0
    lax.fori_loop(0, 2, layer, 0)

    for c in range(8):
        for j in range(5):
            n = min(128, D - 128 * j)
            lo = xres[128 * j:128 * j + n, 128 * c:128 * c + 128].astype(jnp.bfloat16).astype(jnp.float32)
            hi = xres[128 * j:128 * j + n, 1024 + 128 * c:1024 + 128 * c + 128].astype(jnp.bfloat16).astype(jnp.float32)
            wd = (pltpu.bitcast(lo, U32) >> 16) | pltpu.bitcast(hi, U32)
            if n < 128:
                wd = jnp.concatenate([wd, jnp.zeros((128 - n, 128), U32)], axis=0)
            pscr[j, pl.ds(c, 128, stride=8), :] = wd.T
    for p0 in range(0, S, 512):
        parts = [pscr[j, p0 // 2:p0 // 2 + 256, 0:min(128, D - 128 * j)] for j in range(5)]
        words = jnp.concatenate(parts, axis=1)
        xin[:, p0:p0 + 512] = pltpu.bitcast(words, jnp.bfloat16).T
    oc = pltpu.make_async_copy(xin, o_hbm, sems.at[6])
    oc.start()
    oc.wait()


@jax.jit
def pallas_interleave_layers__sliding_local_dilated__glu_gated_geglu__prompt_kernel(
        A_x, A_wqkv, A_wo, B_x, B_w_gate, B_w_up, B_w_down):
    xT = A_x.reshape(S, D).T
    wdT = B_w_down.T
    hbm = pl.BlockSpec(memory_space=pltpu.HBM)
    bf = jnp.bfloat16
    outT = pl.pallas_call(
        _kernel,
        out_shape=jax.ShapeDtypeStruct((D, S), bf),
        in_specs=[hbm] * 6,
        out_specs=hbm,
        scratch_shapes=[
            pltpu.VMEM((D, S), bf),
            pltpu.VMEM((D, 3 * D), bf),
            pltpu.VMEM((D, D), bf),
            pltpu.VMEM((D, F), bf),
            pltpu.VMEM((D, F), bf),
            pltpu.VMEM((D, F), bf),
            pltpu.VMEM((3 * D, D), bf),
            pltpu.VMEM((D, D), bf),
            pltpu.VMEM((D, D), bf),
            pltpu.VMEM((D, S), jnp.float32),
            pltpu.VMEM((8, D, 128), jnp.float32),
            pltpu.VMEM((15, D, 128), jnp.float32),
            pltpu.VMEM((15, D, 128), jnp.float32),
            pltpu.VMEM((D, 1024), jnp.float32),
            pltpu.VMEM((5, 1024, 128), U32),
            pltpu.VMEM((T, D), bf),
            pltpu.SemaphoreType.DMA((7,)),
        ],
        compiler_params=pltpu.CompilerParams(vmem_limit_bytes=100 * 1024 * 1024),
    )(xT, A_wqkv, A_wo, B_w_gate, B_w_up, wdT)
    return outT.T.reshape(1, S, D)
```

```python
import numpy as np
import jax
import jax.numpy as jnp
from jax import lax
import jax.experimental.pallas as pl
import jax.experimental.pallas.tpu as pltpu

S, D, H, DH, F = 2048, 576, 32, 18, 4608
W = 8
T = 1024
T2 = T // 2
FC = 768
H2 = FC // 2
KS = (256, 320, 256, 256, 320, 384, 384)
SWC = 256
SWR = 32
HG = 8
EPS = 1e-5
SCALE = DH ** -0.5
NEG = -1e9 / SCALE
NT = (((1,), (1,)), ((), ()))
U32 = jnp.uint32


def _lnT(x):
    m = jnp.mean(x, axis=0, keepdims=True)
    xc = x - m
    v = jnp.mean(xc * xc, axis=0, keepdims=True)
    return xc * lax.rsqrt(v + EPS)


def _gelu(x):
    c = 0.7978845608028654
    return 0.5 * x * (1.0 + jnp.tanh(c * (x + 0.044715 * (x * x * x))))


def _unpack(w):
    lo = pltpu.bitcast(w << 16, jnp.float32)
    hi = pltpu.bitcast(w & jnp.uint32(0xFFFF0000), jnp.float32)
    return lo, hi


def _attn_slab(qx, kx, vx, obuf, c, ocol):
    lane0 = lax.broadcasted_iota(jnp.int32, (HG, 128), 1) == 0
    for g in range(H // HG):
        acc = [None] * W
        for d in range(DH):
            r = d * H + g * HG
            q = qx[c, pl.ds(r, HG), :]
            for w in range(W):
                p = q * kx[c + 7 - w, pl.ds(r, HG), :]
                acc[w] = p if acc[w] is None else acc[w] + p
        ls = [jnp.where(lane0, NEG, acc[w]) if c < w else acc[w] for w in range(W)]
        m = ls[0]
        for w in range(1, W):
            m = jnp.maximum(m, ls[w])
        es = [jnp.exp((l - m) * SCALE) for l in ls]
        ssum = es[0]
        for w in range(1, W):
            ssum = ssum + es[w]
        inv = 1.0 / ssum
        ps = [e * inv for e in es]
        for d in range(DH):
            r = d * H + g * HG
            o = None
            for w in range(W):
                p = ps[w] * vx[c + 7 - w, pl.ds(r, HG), :]
                o = p if o is None else o + p
            obuf[pl.ds(r, HG), pl.ds(ocol, 128)] = o.astype(obuf.dtype)


def _kernel(xT_hbm, wqkv_hbm, wo_hbm, wg_hbm, wu_hbm, wdT_hbm, o_hbm,
            xin, wqkv, wo, gu7, dn7, wT, woP, woT, xres, qx, kx, vx, obuf, pscr, xa, sems):
    copies = [pltpu.make_async_copy(s, d, sems.at[i]) for i, (s, d) in enumerate(
        ((xT_hbm, xin), (wqkv_hbm, wqkv), (wo_hbm, wo)))]
    for c in copies:
        c.start()
    gu_cp = [pltpu.make_async_copy(s, d, sems.at[3]) for s, d in (
        (wg_hbm.at[0:256], gu7.at[1, 0:256]),
        (wu_hbm.at[0:256], gu7.at[2, 0:256]),
        (wg_hbm.at[256:512], gu7.at[3, 0:256]),
        (wu_hbm.at[256:512], gu7.at[4, 0:256]),
        (wg_hbm.at[512:576], gu7.at[1, 256:320]),
        (wu_hbm.at[512:576], gu7.at[4, 256:320]),
        (wu_hbm.at[512:576], gu7.at[5, 256:320]),
        (wg_hbm.at[512:576], gu7.at[5, 320:384]),
        (wg_hbm.at[512:576], gu7.at[6, 256:320]),
        (wu_hbm.at[512:576], gu7.at[6, 320:384]))]
    dn_cp = []
    for c in range(F // FC):
        f0, h0 = c * FC, c * H2
        for src_r, src_c, slot in ((0, 0, 2), (0, H2, 6), (288, 0, 1), (288, H2, 3)):
            dn_cp.append(pltpu.make_async_copy(
                wdT_hbm.at[src_r:src_r + 288, f0 + src_c:f0 + src_c + H2],
                dn7.at[slot, :, h0:h0 + H2], sems.at[4]))
    for c in gu_cp + dn_cp:
        c.start()

    copies[0].wait()
    for p0 in range(0, S, 512):
        words = pltpu.bitcast(xin[:, p0:p0 + 512].T, U32)
        for j in range(5):
            n = min(128, D - 128 * j)
            pscr[j, p0 // 2:p0 // 2 + 256, 0:n] = words[:, 128 * j:128 * j + n]
    for c in range(8):
        for j in range(5):
            n = min(128, D - 128 * j)
            wt = pscr[j, pl.ds(c, 128, stride=8), :].T
            lo, hi = _unpack(wt[0:n, :])
            xres[128 * j:128 * j + n, 128 * c:128 * c + 128] = lo
            xres[128 * j:128 * j + n, 1024 + 128 * c:1024 + 128 * c + 128] = hi

    copies[1].wait()
    for i in range(14):
        n = min(128, 3 * D - 128 * i)
        words = pltpu.bitcast(wqkv[:, 128 * i:128 * i + n].T, U32)
        for j in range(5):
            m = min(128, D - 128 * j)
            pscr[j, 64 * i:64 * i + n // 2, 0:m] = words[:, 128 * j:128 * j + m]
    for t in range(3):
        for e in range(9):
            for j in range(5):
                m = min(128, D - 128 * j)
                lo, hi = _unpack(pscr[j, pl.ds(t * 288 + e, 32, stride=9), 0:m])
                wT[t * D + 64 * e:t * D + 64 * e + 64, 128 * j:128 * j + m] = (
                    jnp.concatenate([lo, hi], axis=0).astype(jnp.bfloat16))
    copies[2].wait()
    words = pltpu.bitcast(wo[...], U32)
    for j in range(5):
        m = min(128, D - 128 * j)
        pscr[j, 0:288, 0:m] = words[:, 128 * j:128 * j + m]
    for e in range(9):
        for j in range(5):
            m = min(128, D - 128 * j)
            lo, hi = _unpack(pscr[j, pl.ds(e, 32, stride=9), 0:m])
            woP[64 * e:64 * e + 64, 128 * j:128 * j + m] = jnp.concatenate([lo, hi], axis=0).astype(jnp.bfloat16)
    woT[...] = woP[...].T

    def attn_phase():
        def par(p, _):
            c0 = pl.multiple_of(p * 1024, 1024)
            xnT = _lnT(xres[:, pl.ds(c0, 1024)]).astype(jnp.bfloat16)
            k = jnp.dot(wT[D:2 * D, :], xnT, preferred_element_type=jnp.float32)
            v = jnp.dot(wT[2 * D:3 * D, :], xnT, preferred_element_type=jnp.float32)
            q = jnp.dot(wT[0:D, :], xnT, preferred_element_type=jnp.float32)
            for c in range(8):
                kc = k[:, 128 * c:128 * c + 128]
                vc = v[:, 128 * c:128 * c + 128]
                kx[7 + c] = kc
                vx[7 + c] = vc
                if c >= 1:
                    kx[c - 1] = pltpu.roll(kc, 1, 1)
                    vx[c - 1] = pltpu.roll(vc, 1, 1)
                qx[c] = q[:, 128 * c:128 * c + 128]
            for c in range(8):
                _attn_slab(qx, kx, vx, obuf, c, 128 * c)
            y = jnp.dot(woT[...], obuf[...].astype(jnp.bfloat16), preferred_element_type=jnp.float32)
            xres[:, pl.ds(c0, 1024)] += y
            return 0
        with jax.named_scope("att"):
            lax.fori_loop(0, 2, par, 0)

    def strassen_weights():
        for c in gu_cp + dn_cp:
            c.wait()
        f32 = jnp.float32
        bf = jnp.bfloat16

        def gu_body(i, _):
            cs = pl.ds(pl.multiple_of(i * SWC, SWC), SWC)
            for r in range(0, 256, SWR):
                rs = slice(r, r + SWR)
                b11 = gu7[1, rs, cs].astype(f32)
                b12 = gu7[2, rs, cs].astype(f32)
                b21 = gu7[3, rs, cs].astype(f32)
                b22 = gu7[4, rs, cs].astype(f32)
                gu7[0, rs, cs] = (b11 + b22).astype(bf)
                gu7[2, rs, cs] = (b12 - b22).astype(bf)
                gu7[3, rs, cs] = (b21 - b11).astype(bf)
                gu7[5, rs, cs] = (b11 + b12).astype(bf)
                gu7[6, rs, cs] = (b21 + b22).astype(bf)
            return 0
        lax.fori_loop(0, F // SWC, gu_body, 0)

        def dn_body(i, _):
            cs = pl.ds(pl.multiple_of(i * SWC, SWC), SWC)
            for r in range(0, 288, SWR):
                rs = slice(r, r + SWR)
                a11 = dn7[2, rs, cs].astype(f32)
                a12 = dn7[6, rs, cs].astype(f32)
                a21 = dn7[1, rs, cs].astype(f32)
                a22 = dn7[3, rs, cs].astype(f32)
                dn7[0, rs, cs] = (a11 + a22).astype(bf)
                dn7[1, rs, cs] = (a21 + a22).astype(bf)
                dn7[4, rs, cs] = (a11 + a12).astype(bf)
                dn7[5, rs, cs] = (a21 - a11).astype(bf)
                dn7[6, rs, cs] = (a12 - a22).astype(bf)
            return 0
        lax.fori_loop(0, F // 2 // SWC, dn_body, 0)

    def ffn_phase():
        def dot(a, b):
            return jnp.dot(a, b, preferred_element_type=jnp.float32)

        def tile(i, _):
            c0 = pl.multiple_of(i * T, T)
            xr = xres[:, pl.ds(c0, T)]
            xn = _lnT(xr).astype(jnp.bfloat16).T.astype(jnp.float32)
            a11, a12, a21, a22 = xn[:T2, 0:256], xn[:T2, 256:512], xn[T2:, 0:256], xn[T2:, 256:512]
            at, ab = xn[:T2, 512:576], xn[T2:, 512:576]
            bf = jnp.bfloat16
            cc = lambda *a: jnp.concatenate(a, axis=1)
            for k, a in enumerate((a11 + a22, cc(a21 + a22, ab), a11, a22, cc(a11 + a12, at),
                                   cc(a21 - a11, ab, ab), cc(a12 - a22, at, at))):
                xa[k, :, 0:KS[k]] = a.astype(bf)

            def chunk(c, _):
                f0 = pl.multiple_of(c * FC, FC)
                h0 = pl.multiple_of(c * H2, H2)
                G = lambda k: dot(xa[k, :, 0:KS[k]], gu7[k, 0:KS[k], pl.ds(f0, FC)])
                Dn = lambda k, b: lax.dot_general(dn7[k, :, pl.ds(h0, H2)], b.astype(bf), NT,
                                                  preferred_element_type=jnp.float32)
                m1 = G(0); m4 = G(3); m5 = G(4); m7 = G(6)
                g1 = m1 + m4 - m5 + m7
                m3 = G(2)
                u1 = m3 + m5
                h1 = _gelu(g1) * u1
                m2 = G(1)
                g2 = m2 + m4
                m6 = G(5)
                u2 = m1 - m2 + m3 + m6
                h2 = _gelu(g2) * u2
                b11, b21 = h1[:, :H2], h1[:, H2:]
                b12, b22 = h2[:, :H2], h2[:, H2:]
                n2 = Dn(1, b11); n4 = Dn(3, b21 - b11)
                c21 = n2 + n4
                n5 = Dn(4, b22); n3 = Dn(2, b12 - b22)
                c12 = n3 + n5
                n1 = Dn(0, b11 + b22); n7 = Dn(6, b21 + b22)
                c11 = n1 + n4 - n5 + n7
                n6 = Dn(5, b11 + b12)
                c22 = n1 - n2 + n3 + n6
                y = jnp.concatenate([cc(c11, c12), cc(c21, c22)], axis=0)
                xres[:, pl.ds(c0, T)] += y
                return 0
            lax.fori_loop(0, F // FC, chunk, 0)
            return 0
        with jax.named_scope("ffn"):
            lax.fori_loop(0, S // T, tile, 0)

    def layer(l, _):
        attn_phase()

        @pl.when(l == 0)
        def _():
            with jax.named_scope("sw"):
                strassen_weights()
        ffn_phase()
        return 0
    lax.fori_loop(0, 2, layer, 0)

    for c in range(8):
        for j in range(5):
            n = min(128, D - 128 * j)
            lo = xres[128 * j:128 * j + n, 128 * c:128 * c + 128].astype(jnp.bfloat16).astype(jnp.float32)
            hi = xres[128 * j:128 * j + n, 1024 + 128 * c:1024 + 128 * c + 128].astype(jnp.bfloat16).astype(jnp.float32)
            wd = (pltpu.bitcast(lo, U32) >> 16) | pltpu.bitcast(hi, U32)
            if n < 128:
                wd = jnp.concatenate([wd, jnp.zeros((128 - n, 128), U32)], axis=0)
            pscr[j, pl.ds(c, 128, stride=8), :] = wd.T
    for p0 in range(0, S, 512):
        parts = [pscr[j, p0 // 2:p0 // 2 + 256, 0:min(128, D - 128 * j)] for j in range(5)]
        words = jnp.concatenate(parts, axis=1)
        xin[:, p0:p0 + 512] = pltpu.bitcast(words, jnp.bfloat16).T
    oc = pltpu.make_async_copy(xin, o_hbm, sems.at[6])
    oc.start()
    oc.wait()


@jax.jit
def pallas_interleave_layers__sliding_local_dilated__glu_gated_geglu__prompt_kernel(
        A_x, A_wqkv, A_wo, B_x, B_w_gate, B_w_up, B_w_down):
    xT = A_x.reshape(S, D).T
    wdT = B_w_down.T
    hbm = pl.BlockSpec(memory_space=pltpu.HBM)
    bf = jnp.bfloat16
    outT = pl.pallas_call(
        _kernel,
        out_shape=jax.ShapeDtypeStruct((D, S), bf),
        in_specs=[hbm] * 6,
        out_specs=hbm,
        scratch_shapes=[
            pltpu.VMEM((D, S), bf),
            pltpu.VMEM((D, 3 * D), bf),
            pltpu.VMEM((D, D), bf),
            pltpu.VMEM((7, 384, F), bf),
            pltpu.VMEM((7, 288, F // 2), bf),
            pltpu.VMEM((3 * D, D), bf),
            pltpu.VMEM((D, D), bf),
            pltpu.VMEM((D, D), bf),
            pltpu.VMEM((D, S), jnp.float32),
            pltpu.VMEM((8, D, 128), jnp.float32),
            pltpu.VMEM((15, D, 128), jnp.float32),
            pltpu.VMEM((15, D, 128), jnp.float32),
            pltpu.VMEM((D, 1024), jnp.float32),
            pltpu.VMEM((5, 1024, 128), U32),
            pltpu.VMEM((7, T2, 384), bf),
            pltpu.SemaphoreType.DMA((7,)),
        ],
        compiler_params=pltpu.CompilerParams(vmem_limit_bytes=100 * 1024 * 1024),
    )(xT, A_wqkv, A_wo, B_w_gate, B_w_up, wdT)
    return outT.T.reshape(1, S, D)
```

```python
import numpy as np
import jax
import jax.numpy as jnp
from jax import lax
import jax.experimental.pallas as pl
import jax.experimental.pallas.tpu as pltpu

S, D, H, DH, F = 2048, 576, 32, 18, 4608
W = 8
T = 2048
T2 = T // 2
FC = 512
H2 = FC // 2
KS = (256, 320, 256, 256, 320, 384, 384)
SWC = 256
SWR = 32
HG = 8
EPS = 1e-5
SCALE = DH ** -0.5
NEG = -1e9 / SCALE
NT = (((1,), (1,)), ((), ()))
U32 = jnp.uint32


def _lnT(x):
    m = jnp.mean(x, axis=0, keepdims=True)
    xc = x - m
    v = jnp.mean(xc * xc, axis=0, keepdims=True)
    return xc * lax.rsqrt(v + EPS)


def _gelu(x):
    c = 0.7978845608028654
    return 0.5 * x * (1.0 + jnp.tanh(c * (x + 0.044715 * (x * x * x))))


def _unpack(w):
    lo = pltpu.bitcast(w << 16, jnp.float32)
    hi = pltpu.bitcast(w & jnp.uint32(0xFFFF0000), jnp.float32)
    return lo, hi


def _attn_slab(qx, kx, vx, obuf, c, ocol):
    lane0 = lax.broadcasted_iota(jnp.int32, (HG, 128), 1) == 0
    for g in range(H // HG):
        acc = [None] * W
        for d in range(DH):
            r = d * H + g * HG
            q = qx[c, pl.ds(r, HG), :]
            for w in range(W):
                p = q * kx[c + 7 - w, pl.ds(r, HG), :]
                acc[w] = p if acc[w] is None else acc[w] + p
        ls = [jnp.where(lane0, NEG, acc[w]) if c < w else acc[w] for w in range(W)]
        m = ls[0]
        for w in range(1, W):
            m = jnp.maximum(m, ls[w])
        es = [jnp.exp((l - m) * SCALE) for l in ls]
        ssum = es[0]
        for w in range(1, W):
            ssum = ssum + es[w]
        inv = 1.0 / ssum
        ps = [e * inv for e in es]
        for d in range(DH):
            r = d * H + g * HG
            o = None
            for w in range(W):
                p = ps[w] * vx[c + 7 - w, pl.ds(r, HG), :]
                o = p if o is None else o + p
            obuf[pl.ds(r, HG), pl.ds(ocol, 128)] = o.astype(obuf.dtype)


def _kernel(xT_hbm, wqkv_hbm, wo_hbm, wg_hbm, wu_hbm, wdT_hbm, o_hbm,
            xin, wqkv, wo, gu7, dn7, wT, woP, woT, xres, qx, kx, vx, obuf, pscr, xa, sems):
    XC = 512
    x_cp = [pltpu.make_async_copy(xT_hbm.at[:, p0:p0 + XC], xin.at[:, p0:p0 + XC], sems.at[i])
            for i, p0 in enumerate(range(0, S, XC))]
    wqkv_cp = pltpu.make_async_copy(wqkv_hbm, wqkv, sems.at[4])
    wo_cp = pltpu.make_async_copy(wo_hbm, wo, sems.at[5])
    for c in x_cp + [wqkv_cp, wo_cp]:
        c.start()
    gu_cp = [pltpu.make_async_copy(s, d, sems.at[6]) for s, d in (
        (wg_hbm.at[0:256], gu7.at[1, 0:256]),
        (wu_hbm.at[0:256], gu7.at[2, 0:256]),
        (wg_hbm.at[256:512], gu7.at[3, 0:256]),
        (wu_hbm.at[256:512], gu7.at[4, 0:256]),
        (wg_hbm.at[512:576], gu7.at[1, 256:320]),
        (wu_hbm.at[512:576], gu7.at[4, 256:320]),
        (wu_hbm.at[512:576], gu7.at[5, 256:320]),
        (wg_hbm.at[512:576], gu7.at[5, 320:384]),
        (wg_hbm.at[512:576], gu7.at[6, 256:320]),
        (wu_hbm.at[512:576], gu7.at[6, 320:384]))]
    dn_cp = []
    for c in range(F // FC):
        f0, h0 = c * FC, c * H2
        for src_r, src_c, slot in ((0, 0, 2), (0, H2, 6), (288, 0, 1), (288, H2, 3)):
            dn_cp.append(pltpu.make_async_copy(
                wdT_hbm.at[src_r:src_r + 288, f0 + src_c:f0 + src_c + H2],
                dn7.at[slot, :, h0:h0 + H2], sems.at[7]))
    for c in gu_cp + dn_cp:
        c.start()

    for i, p0 in enumerate(range(0, S, XC)):
        x_cp[i].wait()
        words = pltpu.bitcast(xin[:, p0:p0 + 512].T, U32)
        for j in range(5):
            n = min(128, D - 128 * j)
            pscr[j, p0 // 2:p0 // 2 + 256, 0:n] = words[:, 128 * j:128 * j + n]
    for c in range(8):
        for j in range(5):
            n = min(128, D - 128 * j)
            wt = pscr[j, pl.ds(c, 128, stride=8), :].T
            lo, hi = _unpack(wt[0:n, :])
            xres[128 * j:128 * j + n, 128 * c:128 * c + 128] = lo
            xres[128 * j:128 * j + n, 1024 + 128 * c:1024 + 128 * c + 128] = hi

    wqkv_cp.wait()
    for i in range(14):
        n = min(128, 3 * D - 128 * i)
        words = pltpu.bitcast(wqkv[:, 128 * i:128 * i + n].T, U32)
        for j in range(5):
            m = min(128, D - 128 * j)
            pscr[j, 64 * i:64 * i + n // 2, 0:m] = words[:, 128 * j:128 * j + m]
    for t in range(3):
        for e in range(9):
            for j in range(5):
                m = min(128, D - 128 * j)
                lo, hi = _unpack(pscr[j, pl.ds(t * 288 + e, 32, stride=9), 0:m])
                wT[t * D + 64 * e:t * D + 64 * e + 64, 128 * j:128 * j + m] = (
                    jnp.concatenate([lo, hi], axis=0).astype(jnp.bfloat16))
    wo_cp.wait()
    words = pltpu.bitcast(wo[...], U32)
    for j in range(5):
        m = min(128, D - 128 * j)
        pscr[j, 0:288, 0:m] = words[:, 128 * j:128 * j + m]
    for e in range(9):
        for j in range(5):
            m = min(128, D - 128 * j)
            lo, hi = _unpack(pscr[j, pl.ds(e, 32, stride=9), 0:m])
            woP[64 * e:64 * e + 64, 128 * j:128 * j + m] = jnp.concatenate([lo, hi], axis=0).astype(jnp.bfloat16)
    woT[...] = woP[...].T

    def attn_phase():
        def par(p, _):
            c0 = pl.multiple_of(p * 1024, 1024)
            xnT = _lnT(xres[:, pl.ds(c0, 1024)]).astype(jnp.bfloat16)
            k = jnp.dot(wT[D:2 * D, :], xnT, preferred_element_type=jnp.float32)
            v = jnp.dot(wT[2 * D:3 * D, :], xnT, preferred_element_type=jnp.float32)
            q = jnp.dot(wT[0:D, :], xnT, preferred_element_type=jnp.float32)
            for c in range(8):
                kc = k[:, 128 * c:128 * c + 128]
                vc = v[:, 128 * c:128 * c + 128]
                kx[7 + c] = kc
                vx[7 + c] = vc
                if c >= 1:
                    kx[c - 1] = pltpu.roll(kc, 1, 1)
                    vx[c - 1] = pltpu.roll(vc, 1, 1)
                qx[c] = q[:, 128 * c:128 * c + 128]
            for c in range(8):
                _attn_slab(qx, kx, vx, obuf, c, 128 * c)
            y = jnp.dot(woT[...], obuf[...].astype(jnp.bfloat16), preferred_element_type=jnp.float32)
            xres[:, pl.ds(c0, 1024)] += y
            return 0
        with jax.named_scope("att"):
            lax.fori_loop(0, 2, par, 0)

    def strassen_weights():
        for c in gu_cp + dn_cp:
            c.wait()
        f32 = jnp.float32
        bf = jnp.bfloat16

        def gu_body(i, _):
            cs = pl.ds(pl.multiple_of(i * SWC, SWC), SWC)
            for r in range(0, 256, SWR):
                rs = slice(r, r + SWR)
                b11 = gu7[1, rs, cs].astype(f32)
                b12 = gu7[2, rs, cs].astype(f32)
                b21 = gu7[3, rs, cs].astype(f32)
                b22 = gu7[4, rs, cs].astype(f32)
                gu7[0, rs, cs] = (b11 + b22).astype(bf)
                gu7[2, rs, cs] = (b12 - b22).astype(bf)
                gu7[3, rs, cs] = (b21 - b11).astype(bf)
                gu7[5, rs, cs] = (b11 + b12).astype(bf)
                gu7[6, rs, cs] = (b21 + b22).astype(bf)
            return 0
        lax.fori_loop(0, F // SWC, gu_body, 0)

        def dn_body(i, _):
            cs = pl.ds(pl.multiple_of(i * SWC, SWC), SWC)
            for r in range(0, 288, SWR):
                rs = slice(r, r + SWR)
                a11 = dn7[2, rs, cs].astype(f32)
                a12 = dn7[6, rs, cs].astype(f32)
                a21 = dn7[1, rs, cs].astype(f32)
                a22 = dn7[3, rs, cs].astype(f32)
                dn7[0, rs, cs] = (a11 + a22).astype(bf)
                dn7[1, rs, cs] = (a21 + a22).astype(bf)
                dn7[4, rs, cs] = (a11 + a12).astype(bf)
                dn7[5, rs, cs] = (a21 - a11).astype(bf)
                dn7[6, rs, cs] = (a12 - a22).astype(bf)
            return 0
        lax.fori_loop(0, F // 2 // SWC, dn_body, 0)

    def ffn_phase():
        def dot(a, b):
            return jnp.dot(a, b, preferred_element_type=jnp.float32)

        def tile(i, _):
            c0 = pl.multiple_of(i * T, T)
            xr = xres[:, pl.ds(c0, T)]
            xn = _lnT(xr).astype(jnp.bfloat16).T.astype(jnp.float32)
            a11, a12, a21, a22 = xn[:T2, 0:256], xn[:T2, 256:512], xn[T2:, 0:256], xn[T2:, 256:512]
            at, ab = xn[:T2, 512:576], xn[T2:, 512:576]
            bf = jnp.bfloat16
            cc = lambda *a: jnp.concatenate(a, axis=1)
            for k, a in enumerate((a11 + a22, cc(a21 + a22, ab), a11, a22, cc(a11 + a12, at),
                                   cc(a21 - a11, ab, ab), cc(a12 - a22, at, at))):
                xa[k, :, 0:KS[k]] = a.astype(bf)

            def chunk(c, _):
                f0 = pl.multiple_of(c * FC, FC)
                h0 = pl.multiple_of(c * H2, H2)
                G = lambda k: dot(xa[k, :, 0:KS[k]], gu7[k, 0:KS[k], pl.ds(f0, FC)])
                Dn = lambda k, b: lax.dot_general(dn7[k, :, pl.ds(h0, H2)], b.astype(bf), NT,
                                                  preferred_element_type=jnp.float32)
                m1 = G(0); m4 = G(3); m5 = G(4); m7 = G(6)
                g1 = m1 + m4 - m5 + m7
                m3 = G(2)
                u1 = m3 + m5
                h1 = _gelu(g1) * u1
                m2 = G(1)
                g2 = m2 + m4
                m6 = G(5)
                u2 = m1 - m2 + m3 + m6
                h2 = _gelu(g2) * u2
                b11, b21 = h1[:, :H2], h1[:, H2:]
                b12, b22 = h2[:, :H2], h2[:, H2:]
                n2 = Dn(1, b11); n4 = Dn(3, b21 - b11)
                c21 = n2 + n4
                n5 = Dn(4, b22); n3 = Dn(2, b12 - b22)
                c12 = n3 + n5
                n1 = Dn(0, b11 + b22); n7 = Dn(6, b21 + b22)
                c11 = n1 + n4 - n5 + n7
                n6 = Dn(5, b11 + b12)
                c22 = n1 - n2 + n3 + n6
                y = jnp.concatenate([cc(c11, c12), cc(c21, c22)], axis=0)
                xres[:, pl.ds(c0, T)] += y
                return 0
            lax.fori_loop(0, F // FC, chunk, 0)
            return 0
        with jax.named_scope("ffn"):
            lax.fori_loop(0, S // T, tile, 0)

    def layer(l, _):
        attn_phase()

        @pl.when(l == 0)
        def _():
            with jax.named_scope("sw"):
                strassen_weights()
        ffn_phase()
        return 0
    lax.fori_loop(0, 2, layer, 0)

    out_cp = []
    for j in range(5):
        n = min(128, D - 128 * j)
        rs = slice(128 * j, 128 * j + n)
        for c in range(8):
            lo = xres[rs, 128 * c:128 * c + 128].astype(jnp.bfloat16).astype(jnp.float32)
            hi = xres[rs, 1024 + 128 * c:1024 + 128 * c + 128].astype(jnp.bfloat16).astype(jnp.float32)
            wd = (pltpu.bitcast(lo, U32) >> 16) | pltpu.bitcast(hi, U32)
            if n < 128:
                wd = jnp.concatenate([wd, jnp.zeros((128 - n, 128), U32)], axis=0)
            pscr[j, pl.ds(c, 128, stride=8), :] = wd.T
        xt = pltpu.bitcast(pscr[j], jnp.bfloat16).T
        xin[rs, :] = xt[0:n, :]
        cp = pltpu.make_async_copy(xin.at[rs], o_hbm.at[rs], sems.at[j])
        cp.start()
        out_cp.append(cp)
    for cp in out_cp:
        cp.wait()


@jax.jit
def pallas_interleave_layers__sliding_local_dilated__glu_gated_geglu__prompt_kernel(
        A_x, A_wqkv, A_wo, B_x, B_w_gate, B_w_up, B_w_down):
    xT = A_x.reshape(S, D).T
    wdT = B_w_down.T
    hbm = pl.BlockSpec(memory_space=pltpu.HBM)
    bf = jnp.bfloat16
    outT = pl.pallas_call(
        _kernel,
        out_shape=jax.ShapeDtypeStruct((D, S), bf),
        in_specs=[hbm] * 6,
        out_specs=hbm,
        scratch_shapes=[
            pltpu.VMEM((D, S), bf),
            pltpu.VMEM((D, 3 * D), bf),
            pltpu.VMEM((D, D), bf),
            pltpu.VMEM((7, 384, F), bf),
            pltpu.VMEM((7, 288, F // 2), bf),
            pltpu.VMEM((3 * D, D), bf),
            pltpu.VMEM((D, D), bf),
            pltpu.VMEM((D, D), bf),
            pltpu.VMEM((D, S), jnp.float32),
            pltpu.VMEM((8, D, 128), jnp.float32),
            pltpu.VMEM((15, D, 128), jnp.float32),
            pltpu.VMEM((15, D, 128), jnp.float32),
            pltpu.VMEM((D, 1024), jnp.float32),
            pltpu.VMEM((5, 1024, 128), U32),
            pltpu.VMEM((7, T2, 384), bf),
            pltpu.SemaphoreType.DMA((8,)),
        ],
        compiler_params=pltpu.CompilerParams(vmem_limit_bytes=100 * 1024 * 1024),
    )(xT, A_wqkv, A_wo, B_w_gate, B_w_up, wdT)
    return outT.T.reshape(1, S, D)
```

```python
import numpy as np
import jax
import jax.numpy as jnp
from jax import lax
import jax.experimental.pallas as pl
import jax.experimental.pallas.tpu as pltpu

S, D, H, DH, F = 2048, 576, 32, 18, 4608
W = 8
T = 2048
T2 = T // 2
FC = 512
H2 = FC // 2
KS = (256, 320, 256, 256, 320, 384, 384)
SWC = 256
SWR = 32
PR = 256
PLOOP = False
PMODE = 0
HG = 8
EPS = 1e-5
SCALE = DH ** -0.5
NEG = -1e9 / SCALE
NT = (((1,), (1,)), ((), ()))
U32 = jnp.uint32


def _lnT(x):
    m = jnp.mean(x, axis=0, keepdims=True)
    xc = x - m
    v = jnp.mean(xc * xc, axis=0, keepdims=True)
    return xc * lax.rsqrt(v + EPS)


def _gelu(x):
    c = 0.7978845608028654
    return 0.5 * x * (1.0 + jnp.tanh(c * (x + 0.044715 * (x * x * x))))


def _unpack(w):
    lo = pltpu.bitcast(w << 16, jnp.float32)
    hi = pltpu.bitcast(w & jnp.uint32(0xFFFF0000), jnp.float32)
    return lo, hi


def _attn_slab(qx, kx, vx, obuf, c, ocol):
    lane0 = lax.broadcasted_iota(jnp.int32, (HG, 128), 1) == 0
    for g in range(H // HG):
        acc = [None] * W
        for d in range(DH):
            r = d * H + g * HG
            q = qx[c, pl.ds(r, HG), :]
            for w in range(W):
                p = q * kx[c + 7 - w, pl.ds(r, HG), :]
                acc[w] = p if acc[w] is None else acc[w] + p
        ls = [jnp.where(lane0, NEG, acc[w]) if c < w else acc[w] for w in range(W)]
        m = ls[0]
        for w in range(1, W):
            m = jnp.maximum(m, ls[w])
        es = [jnp.exp((l - m) * SCALE) for l in ls]
        ssum = es[0]
        for w in range(1, W):
            ssum = ssum + es[w]
        inv = 1.0 / ssum
        ps = [e * inv for e in es]
        for d in range(DH):
            r = d * H + g * HG
            o = None
            for w in range(W):
                p = ps[w] * vx[c + 7 - w, pl.ds(r, HG), :]
                o = p if o is None else o + p
            obuf[pl.ds(r, HG), pl.ds(ocol, 128)] = o.astype(obuf.dtype)


def _kernel(xT_hbm, wqkv_hbm, wo_hbm, wg_hbm, wu_hbm, wdT_hbm, o_hbm,
            xin, wqkv, wo, gu7, dn7, wT, woP, woT, xres, qx, kx, vx, obuf, pscr, xa, sems):
    XC = 512
    x_cp = [pltpu.make_async_copy(xT_hbm.at[:, p0:p0 + XC], xin.at[:, p0:p0 + XC], sems.at[i])
            for i, p0 in enumerate(range(0, S, XC))]
    wqkv_cp = pltpu.make_async_copy(wqkv_hbm, wqkv, sems.at[4])
    wo_cp = pltpu.make_async_copy(wo_hbm, wo, sems.at[5])
    for c in x_cp + [wqkv_cp, wo_cp]:
        c.start()
    gu_cp = [pltpu.make_async_copy(s, d, sems.at[6]) for s, d in (
        (wg_hbm.at[0:256], gu7.at[1, 0:256]),
        (wu_hbm.at[0:256], gu7.at[2, 0:256]),
        (wg_hbm.at[256:512], gu7.at[3, 0:256]),
        (wu_hbm.at[256:512], gu7.at[4, 0:256]),
        (wg_hbm.at[512:576], gu7.at[1, 256:320]),
        (wu_hbm.at[512:576], gu7.at[4, 256:320]),
        (wu_hbm.at[512:576], gu7.at[5, 256:320]),
        (wg_hbm.at[512:576], gu7.at[5, 320:384]),
        (wg_hbm.at[512:576], gu7.at[6, 256:320]),
        (wu_hbm.at[512:576], gu7.at[6, 320:384]))]
    dn_cp = []
    for c in range(F // FC):
        f0, h0 = c * FC, c * H2
        for src_r, src_c, slot in ((0, 0, 2), (0, H2, 6), (288, 0, 1), (288, H2, 3)):
            dn_cp.append(pltpu.make_async_copy(
                wdT_hbm.at[src_r:src_r + 288, f0 + src_c:f0 + src_c + H2],
                dn7.at[slot, :, h0:h0 + H2], sems.at[7]))
    for c in gu_cp + dn_cp:
        c.start()

    for i, p0 in enumerate(range(0, S, XC)):
        x_cp[i].wait()
        words = pltpu.bitcast(xin[:, p0:p0 + 512].T, U32)
        for j in range(5):
            n = min(128, D - 128 * j)
            pscr[j, p0 // 2:p0 // 2 + 256, 0:n] = words[:, 128 * j:128 * j + n]
    for c in range(8):
        for j in range(5):
            n = min(128, D - 128 * j)
            wt = pscr[j, pl.ds(c, 128, stride=8), :].T
            lo, hi = _unpack(wt[0:n, :])
            xres[128 * j:128 * j + n, 128 * c:128 * c + 128] = lo
            xres[128 * j:128 * j + n, 1024 + 128 * c:1024 + 128 * c + 128] = hi

    wqkv_cp.wait()
    for i in range(14):
        n = min(128, 3 * D - 128 * i)
        words = pltpu.bitcast(wqkv[:, 128 * i:128 * i + n].T, U32)
        for j in range(5):
            m = min(128, D - 128 * j)
            pscr[j, 64 * i:64 * i + n // 2, 0:m] = words[:, 128 * j:128 * j + m]
    for t in range(3):
        for e in range(9):
            for j in range(5):
                m = min(128, D - 128 * j)
                lo, hi = _unpack(pscr[j, pl.ds(t * 288 + e, 32, stride=9), 0:m])
                wT[t * D + 64 * e:t * D + 64 * e + 64, 128 * j:128 * j + m] = (
                    jnp.concatenate([lo, hi], axis=0).astype(jnp.bfloat16))
    wo_cp.wait()
    words = pltpu.bitcast(wo[...], U32)
    for j in range(5):
        m = min(128, D - 128 * j)
        pscr[j, 0:288, 0:m] = words[:, 128 * j:128 * j + m]
    for e in range(9):
        for j in range(5):
            m = min(128, D - 128 * j)
            lo, hi = _unpack(pscr[j, pl.ds(e, 32, stride=9), 0:m])
            woP[64 * e:64 * e + 64, 128 * j:128 * j + m] = jnp.concatenate([lo, hi], axis=0).astype(jnp.bfloat16)
    woT[...] = woP[...].T

    def attn_phase():
        def par(p, _):
            c0 = pl.multiple_of(p * 1024, 1024)
            xnT = _lnT(xres[:, pl.ds(c0, 1024)]).astype(jnp.bfloat16)
            k = jnp.dot(wT[D:2 * D, :], xnT, preferred_element_type=jnp.float32)
            v = jnp.dot(wT[2 * D:3 * D, :], xnT, preferred_element_type=jnp.float32)
            q = jnp.dot(wT[0:D, :], xnT, preferred_element_type=jnp.float32)
            for c in range(8):
                kc = k[:, 128 * c:128 * c + 128]
                vc = v[:, 128 * c:128 * c + 128]
                kx[7 + c] = kc
                vx[7 + c] = vc
                if c >= 1:
                    kx[c - 1] = pltpu.roll(kc, 1, 1)
                    vx[c - 1] = pltpu.roll(vc, 1, 1)
                qx[c] = q[:, 128 * c:128 * c + 128]
            for c in range(8):
                _attn_slab(qx, kx, vx, obuf, c, 128 * c)
            y = jnp.dot(woT[...], obuf[...].astype(jnp.bfloat16), preferred_element_type=jnp.float32)
            xres[:, pl.ds(c0, 1024)] += y
            return 0
        with jax.named_scope("att"):
            lax.fori_loop(0, 2, par, 0)

    def strassen_weights():
        for c in gu_cp + dn_cp:
            c.wait()
        f32 = jnp.float32
        bf = jnp.bfloat16

        def gu_body(i, _):
            cs = pl.ds(pl.multiple_of(i * SWC, SWC), SWC)
            for r in range(0, 256, SWR):
                rs = slice(r, r + SWR)
                b11 = gu7[1, rs, cs].astype(f32)
                b12 = gu7[2, rs, cs].astype(f32)
                b21 = gu7[3, rs, cs].astype(f32)
                b22 = gu7[4, rs, cs].astype(f32)
                gu7[0, rs, cs] = (b11 + b22).astype(bf)
                gu7[2, rs, cs] = (b12 - b22).astype(bf)
                gu7[3, rs, cs] = (b21 - b11).astype(bf)
                gu7[5, rs, cs] = (b11 + b12).astype(bf)
                gu7[6, rs, cs] = (b21 + b22).astype(bf)
            return 0
        lax.fori_loop(0, F // SWC, gu_body, 0)

        def dn_body(i, _):
            cs = pl.ds(pl.multiple_of(i * SWC, SWC), SWC)
            for r in range(0, 288, SWR):
                rs = slice(r, r + SWR)
                a11 = dn7[2, rs, cs].astype(f32)
                a12 = dn7[6, rs, cs].astype(f32)
                a21 = dn7[1, rs, cs].astype(f32)
                a22 = dn7[3, rs, cs].astype(f32)
                dn7[0, rs, cs] = (a11 + a22).astype(bf)
                dn7[1, rs, cs] = (a21 + a22).astype(bf)
                dn7[4, rs, cs] = (a11 + a12).astype(bf)
                dn7[5, rs, cs] = (a21 - a11).astype(bf)
                dn7[6, rs, cs] = (a12 - a22).astype(bf)
            return 0
        lax.fori_loop(0, F // 2 // SWC, dn_body, 0)

    def ffn_phase():
        def dot(a, b):
            return jnp.dot(a, b, preferred_element_type=jnp.float32)

        def tile(i, _):
            c0 = pl.multiple_of(i * T, T)
            bf = jnp.bfloat16
            cc = lambda *a: jnp.concatenate(a, axis=1)

            def prep(r0):
                rs = pl.ds(r0, PR)
                if PMODE == 0:
                    xe = _lnT(xres[:, pl.ds(c0 + r0, PR)]).astype(bf).T.astype(jnp.float32)
                    xo = _lnT(xres[:, pl.ds(c0 + T2 + r0, PR)]).astype(bf).T.astype(jnp.float32)
                    a11, a12, a21, a22 = xe[:, 0:256], xe[:, 256:512], xo[:, 0:256], xo[:, 256:512]
                    at, ab = xe[:, 512:576], xo[:, 512:576]
                    for k, a in enumerate((a11 + a22, cc(a21 + a22, ab), a11, a22, cc(a11 + a12, at),
                                           cc(a21 - a11, ab, ab), cc(a12 - a22, at, at))):
                        xa[k, rs, 0:KS[k]] = a.astype(bf)
                else:
                    xe = _lnT(xres[:, pl.ds(c0 + r0, PR)]).astype(bf).astype(jnp.float32)
                    xo = _lnT(xres[:, pl.ds(c0 + T2 + r0, PR)]).astype(bf).astype(jnp.float32)
                    a11, a12, a21, a22 = xe[0:256], xe[256:512], xo[0:256], xo[256:512]
                    at, ab = xe[512:576], xo[512:576]
                    rc = lambda *a: jnp.concatenate(a, axis=0)
                    for k, a in enumerate((a11 + a22, rc(a21 + a22, ab), a11, a22, rc(a11 + a12, at),
                                           rc(a21 - a11, ab, ab), rc(a12 - a22, at, at))):
                        xa[k, rs, 0:KS[k]] = a.astype(bf).T
            if PLOOP:
                def prep_body(i, _):
                    prep(pl.multiple_of(i * PR, PR))
                    return 0
                lax.fori_loop(0, T2 // PR, prep_body, 0)
            else:
                for r0 in range(0, T2, PR):
                    prep(r0)

            def chunk(c, _):
                f0 = pl.multiple_of(c * FC, FC)
                h0 = pl.multiple_of(c * H2, H2)
                G = lambda k: dot(xa[k, :, 0:KS[k]], gu7[k, 0:KS[k], pl.ds(f0, FC)])
                Dn = lambda k, b: lax.dot_general(dn7[k, :, pl.ds(h0, H2)], b.astype(bf), NT,
                                                  preferred_element_type=jnp.float32)
                m1 = G(0); m4 = G(3); m5 = G(4); m7 = G(6)
                g1 = m1 + m4 - m5 + m7
                m3 = G(2)
                u1 = m3 + m5
                h1 = _gelu(g1) * u1
                m2 = G(1)
                g2 = m2 + m4
                m6 = G(5)
                u2 = m1 - m2 + m3 + m6
                h2 = _gelu(g2) * u2
                b11, b21 = h1[:, :H2], h1[:, H2:]
                b12, b22 = h2[:, :H2], h2[:, H2:]
                n2 = Dn(1, b11); n4 = Dn(3, b21 - b11)
                c21 = n2 + n4
                n5 = Dn(4, b22); n3 = Dn(2, b12 - b22)
                c12 = n3 + n5
                n1 = Dn(0, b11 + b22); n7 = Dn(6, b21 + b22)
                c11 = n1 + n4 - n5 + n7
                n6 = Dn(5, b11 + b12)
                c22 = n1 - n2 + n3 + n6
                y = jnp.concatenate([cc(c11, c12), cc(c21, c22)], axis=0)
                xres[:, pl.ds(c0, T)] += y
                return 0
            lax.fori_loop(0, F // FC, chunk, 0)
            return 0
        with jax.named_scope("ffn"):
            lax.fori_loop(0, S // T, tile, 0)

    def layer(l, _):
        attn_phase()

        @pl.when(l == 0)
        def _():
            with jax.named_scope("sw"):
                strassen_weights()
        ffn_phase()
        return 0
    lax.fori_loop(0, 2, layer, 0)

    out_cp = []
    for j in range(5):
        n = min(128, D - 128 * j)
        rs = slice(128 * j, 128 * j + n)
        for c in range(8):
            lo = xres[rs, 128 * c:128 * c + 128].astype(jnp.bfloat16).astype(jnp.float32)
            hi = xres[rs, 1024 + 128 * c:1024 + 128 * c + 128].astype(jnp.bfloat16).astype(jnp.float32)
            wd = (pltpu.bitcast(lo, U32) >> 16) | pltpu.bitcast(hi, U32)
            if n < 128:
                wd = jnp.concatenate([wd, jnp.zeros((128 - n, 128), U32)], axis=0)
            pscr[j, pl.ds(c, 128, stride=8), :] = wd.T
        xt = pltpu.bitcast(pscr[j], jnp.bfloat16).T
        xin[rs, :] = xt[0:n, :]
        cp = pltpu.make_async_copy(xin.at[rs], o_hbm.at[rs], sems.at[j])
        cp.start()
        out_cp.append(cp)
    for cp in out_cp:
        cp.wait()


@jax.jit
def pallas_interleave_layers__sliding_local_dilated__glu_gated_geglu__prompt_kernel(
        A_x, A_wqkv, A_wo, B_x, B_w_gate, B_w_up, B_w_down):
    xT = A_x.reshape(S, D).T
    wdT = B_w_down.T
    hbm = pl.BlockSpec(memory_space=pltpu.HBM)
    bf = jnp.bfloat16
    outT = pl.pallas_call(
        _kernel,
        out_shape=jax.ShapeDtypeStruct((D, S), bf),
        in_specs=[hbm] * 6,
        out_specs=hbm,
        scratch_shapes=[
            pltpu.VMEM((D, S), bf),
            pltpu.VMEM((D, 3 * D), bf),
            pltpu.VMEM((D, D), bf),
            pltpu.VMEM((7, 384, F), bf),
            pltpu.VMEM((7, 288, F // 2), bf),
            pltpu.VMEM((3 * D, D), bf),
            pltpu.VMEM((D, D), bf),
            pltpu.VMEM((D, D), bf),
            pltpu.VMEM((D, S), jnp.float32),
            pltpu.VMEM((8, D, 128), jnp.float32),
            pltpu.VMEM((15, D, 128), jnp.float32),
            pltpu.VMEM((15, D, 128), jnp.float32),
            pltpu.VMEM((D, 1024), jnp.float32),
            pltpu.VMEM((5, 1024, 128), U32),
            pltpu.VMEM((7, T2, 384), bf),
            pltpu.SemaphoreType.DMA((8,)),
        ],
        compiler_params=pltpu.CompilerParams(vmem_limit_bytes=100 * 1024 * 1024),
    )(xT, A_wqkv, A_wo, B_w_gate, B_w_up, wdT)
    return outT.T.reshape(1, S, D)
```

```python
import jax
import jax.numpy as jnp
from jax import lax
import jax.experimental.pallas as pl
import jax.experimental.pallas.tpu as pltpu

S, D, H, DH, F = 2048, 576, 32, 18, 4608
W = 8
T2 = S // 2
FC = 512
H2 = FC // 2
KS = (256, 320, 256, 256, 320, 384, 384)
SWC, SWR = 256, 32
PR = 256
HG = 8
EPS = 1e-5
SCALE = DH ** -0.5
NEG = -1e9 / SCALE
NT = (((1,), (1,)), ((), ()))
U32 = jnp.uint32


def _lnT(x):
    m = jnp.mean(x, axis=0, keepdims=True)
    xc = x - m
    v = jnp.mean(xc * xc, axis=0, keepdims=True)
    return xc * lax.rsqrt(v + EPS)


def _gelu(x):
    c = 0.7978845608028654
    return 0.5 * x * (1.0 + jnp.tanh(c * (x + 0.044715 * (x * x * x))))


def _unpack(w):
    lo = pltpu.bitcast(w << 16, jnp.float32)
    hi = pltpu.bitcast(w & jnp.uint32(0xFFFF0000), jnp.float32)
    return lo, hi


def _attn_slab(qx, kx, vx, obuf, c, ocol):
    lane0 = lax.broadcasted_iota(jnp.int32, (HG, 128), 1) == 0
    for g in range(H // HG):
        acc = [None] * W
        for d in range(DH):
            r = d * H + g * HG
            q = qx[c, pl.ds(r, HG), :]
            for w in range(W):
                p = q * kx[c + 7 - w, pl.ds(r, HG), :]
                acc[w] = p if acc[w] is None else acc[w] + p
        ls = [jnp.where(lane0, NEG, acc[w]) if c < w else acc[w] for w in range(W)]
        m = ls[0]
        for w in range(1, W):
            m = jnp.maximum(m, ls[w])
        es = [jnp.exp((l - m) * SCALE) for l in ls]
        ssum = es[0]
        for w in range(1, W):
            ssum = ssum + es[w]
        inv = 1.0 / ssum
        ps = [e * inv for e in es]
        for d in range(DH):
            r = d * H + g * HG
            o = None
            for w in range(W):
                p = ps[w] * vx[c + 7 - w, pl.ds(r, HG), :]
                o = p if o is None else o + p
            obuf[pl.ds(r, HG), pl.ds(ocol, 128)] = o.astype(obuf.dtype)


def _kernel(xT_hbm, wqkv_hbm, wo_hbm, wg_hbm, wu_hbm, wdT_hbm, o_hbm,
            xin, wqkv, wo, gu7, dn7, wT, woP, woT, xres, qx, kx, vx, obuf, pscr, xa, sems):
    XC = 512
    x_cp = [pltpu.make_async_copy(xT_hbm.at[:, p0:p0 + XC], xin.at[:, p0:p0 + XC], sems.at[i])
            for i, p0 in enumerate(range(0, S, XC))]
    wqkv_cp = pltpu.make_async_copy(wqkv_hbm, wqkv, sems.at[4])
    wo_cp = pltpu.make_async_copy(wo_hbm, wo, sems.at[5])
    for c in x_cp + [wqkv_cp, wo_cp]:
        c.start()
    gu_cp = [pltpu.make_async_copy(s, d, sems.at[6]) for s, d in (
        (wg_hbm.at[0:256], gu7.at[1, 0:256]),
        (wu_hbm.at[0:256], gu7.at[2, 0:256]),
        (wg_hbm.at[256:512], gu7.at[3, 0:256]),
        (wu_hbm.at[256:512], gu7.at[4, 0:256]),
        (wg_hbm.at[512:576], gu7.at[1, 256:320]),
        (wu_hbm.at[512:576], gu7.at[4, 256:320]),
        (wu_hbm.at[512:576], gu7.at[5, 256:320]),
        (wg_hbm.at[512:576], gu7.at[5, 320:384]),
        (wg_hbm.at[512:576], gu7.at[6, 256:320]),
        (wu_hbm.at[512:576], gu7.at[6, 320:384]))]
    dn_cp = []
    for c in range(F // FC):
        f0, h0 = c * FC, c * H2
        for src_r, src_c, slot in ((0, 0, 2), (0, H2, 6), (288, 0, 1), (288, H2, 3)):
            dn_cp.append(pltpu.make_async_copy(
                wdT_hbm.at[src_r:src_r + 288, f0 + src_c:f0 + src_c + H2],
                dn7.at[slot, :, h0:h0 + H2], sems.at[7]))
    for c in gu_cp + dn_cp:
        c.start()

    pscr[4] = jnp.zeros((1024, 128), U32)
    for i, p0 in enumerate(range(0, S, XC)):
        x_cp[i].wait()
        words = pltpu.bitcast(xin[:, p0:p0 + 512].T, U32)
        for j in range(5):
            n = min(128, D - 128 * j)
            pscr[j, p0 // 2:p0 // 2 + 256, 0:n] = words[:, 128 * j:128 * j + n]
    for c in range(8):
        for j in range(5):
            n = min(128, D - 128 * j)
            wt = pscr[j, pl.ds(c, 128, stride=8), :].T
            lo, hi = _unpack(wt[0:n, :])
            xres[128 * j:128 * j + n, 128 * c:128 * c + 128] = lo
            xres[128 * j:128 * j + n, 1024 + 128 * c:1024 + 128 * c + 128] = hi

    wqkv_cp.wait()
    for i in range(14):
        n = min(128, 3 * D - 128 * i)
        words = pltpu.bitcast(wqkv[:, 128 * i:128 * i + n].T, U32)
        for j in range(5):
            m = min(128, D - 128 * j)
            pscr[j, 64 * i:64 * i + n // 2, 0:m] = words[:, 128 * j:128 * j + m]
    for t in range(3):
        for e in range(9):
            for j in range(5):
                m = min(128, D - 128 * j)
                lo, hi = _unpack(pscr[j, pl.ds(t * 288 + e, 32, stride=9), 0:m])
                wT[t * D + 64 * e:t * D + 64 * e + 64, 128 * j:128 * j + m] = (
                    jnp.concatenate([lo, hi], axis=0).astype(jnp.bfloat16))
    wo_cp.wait()
    words = pltpu.bitcast(wo[...], U32)
    for j in range(5):
        m = min(128, D - 128 * j)
        pscr[j, 0:288, 0:m] = words[:, 128 * j:128 * j + m]
    for e in range(9):
        for j in range(5):
            m = min(128, D - 128 * j)
            lo, hi = _unpack(pscr[j, pl.ds(e, 32, stride=9), 0:m])
            woP[64 * e:64 * e + 64, 128 * j:128 * j + m] = jnp.concatenate([lo, hi], axis=0).astype(jnp.bfloat16)
    woT[...] = woP[...].T

    def attn_phase():
        def par(p, _):
            c0 = pl.multiple_of(p * 1024, 1024)
            xnT = _lnT(xres[:, pl.ds(c0, 1024)]).astype(jnp.bfloat16)
            k = jnp.dot(wT[D:2 * D, :], xnT, preferred_element_type=jnp.float32)
            v = jnp.dot(wT[2 * D:3 * D, :], xnT, preferred_element_type=jnp.float32)
            q = jnp.dot(wT[0:D, :], xnT, preferred_element_type=jnp.float32)
            for c in range(8):
                kc = k[:, 128 * c:128 * c + 128]
                vc = v[:, 128 * c:128 * c + 128]
                kx[7 + c] = kc
                vx[7 + c] = vc
                if c >= 1:
                    kx[c - 1] = pltpu.roll(kc, 1, 1)
                    vx[c - 1] = pltpu.roll(vc, 1, 1)
                qx[c] = q[:, 128 * c:128 * c + 128]
            for c in range(8):
                _attn_slab(qx, kx, vx, obuf, c, 128 * c)
            y = jnp.dot(woT[...], obuf[...].astype(jnp.bfloat16), preferred_element_type=jnp.float32)
            xres[:, pl.ds(c0, 1024)] += y
            return 0
        lax.fori_loop(0, 2, par, 0)

    def strassen_weights():
        for c in gu_cp + dn_cp:
            c.wait()
        f32 = jnp.float32
        bf = jnp.bfloat16

        def gu_body(i, _):
            cs = pl.ds(pl.multiple_of(i * SWC, SWC), SWC)
            for r in range(0, 256, SWR):
                rs = slice(r, r + SWR)
                b11 = gu7[1, rs, cs].astype(f32)
                b12 = gu7[2, rs, cs].astype(f32)
                b21 = gu7[3, rs, cs].astype(f32)
                b22 = gu7[4, rs, cs].astype(f32)
                gu7[0, rs, cs] = (b11 + b22).astype(bf)
                gu7[2, rs, cs] = (b12 - b22).astype(bf)
                gu7[3, rs, cs] = (b21 - b11).astype(bf)
                gu7[5, rs, cs] = (b11 + b12).astype(bf)
                gu7[6, rs, cs] = (b21 + b22).astype(bf)
            return 0
        lax.fori_loop(0, F // SWC, gu_body, 0)

        def dn_body(i, _):
            cs = pl.ds(pl.multiple_of(i * SWC, SWC), SWC)
            for r in range(0, 288, SWR):
                rs = slice(r, r + SWR)
                a11 = dn7[2, rs, cs].astype(f32)
                a12 = dn7[6, rs, cs].astype(f32)
                a21 = dn7[1, rs, cs].astype(f32)
                a22 = dn7[3, rs, cs].astype(f32)
                dn7[0, rs, cs] = (a11 + a22).astype(bf)
                dn7[1, rs, cs] = (a21 + a22).astype(bf)
                dn7[4, rs, cs] = (a11 + a12).astype(bf)
                dn7[5, rs, cs] = (a21 - a11).astype(bf)
                dn7[6, rs, cs] = (a12 - a22).astype(bf)
            return 0
        lax.fori_loop(0, F // 2 // SWC, dn_body, 0)

    def ffn_phase():
        def dot(a, b):
            return jnp.dot(a, b, preferred_element_type=jnp.float32)

        bf = jnp.bfloat16
        cc = lambda *a: jnp.concatenate(a, axis=1)
        for r0 in range(0, T2, PR):
            xe = _lnT(xres[:, r0:r0 + PR]).astype(bf).T.astype(jnp.float32)
            xo = _lnT(xres[:, T2 + r0:T2 + r0 + PR]).astype(bf).T.astype(jnp.float32)
            a11, a12, a21, a22 = xe[:, 0:256], xe[:, 256:512], xo[:, 0:256], xo[:, 256:512]
            at, ab = xe[:, 512:576], xo[:, 512:576]
            for k, a in enumerate((a11 + a22, cc(a21 + a22, ab), a11, a22, cc(a11 + a12, at),
                                   cc(a21 - a11, ab, ab), cc(a12 - a22, at, at))):
                xa[k, r0:r0 + PR, 0:KS[k]] = a.astype(bf)

        def chunk(c, _):
            f0 = pl.multiple_of(c * FC, FC)
            h0 = pl.multiple_of(c * H2, H2)
            G = lambda k: dot(xa[k, :, 0:KS[k]], gu7[k, 0:KS[k], pl.ds(f0, FC)])
            Dn = lambda k, b: lax.dot_general(dn7[k, :, pl.ds(h0, H2)], b.astype(bf), NT,
                                              preferred_element_type=jnp.float32)
            m1 = G(0); m4 = G(3); m5 = G(4); m7 = G(6)
            g1 = m1 + m4 - m5 + m7
            m3 = G(2)
            u1 = m3 + m5
            h1 = _gelu(g1) * u1
            m2 = G(1)
            g2 = m2 + m4
            m6 = G(5)
            u2 = m1 - m2 + m3 + m6
            h2 = _gelu(g2) * u2
            b11, b21 = h1[:, :H2], h1[:, H2:]
            b12, b22 = h2[:, :H2], h2[:, H2:]
            n2 = Dn(1, b11); n4 = Dn(3, b21 - b11)
            c21 = n2 + n4
            n5 = Dn(4, b22); n3 = Dn(2, b12 - b22)
            c12 = n3 + n5
            n1 = Dn(0, b11 + b22); n7 = Dn(6, b21 + b22)
            c11 = n1 + n4 - n5 + n7
            n6 = Dn(5, b11 + b12)
            c22 = n1 - n2 + n3 + n6
            y = jnp.concatenate([cc(c11, c12), cc(c21, c22)], axis=0)
            xres[...] += y
            return 0
        lax.fori_loop(0, F // FC, chunk, 0)

    def layer(l, _):
        attn_phase()

        @pl.when(l == 0)
        def _():
            strassen_weights()
        ffn_phase()
        return 0
    lax.fori_loop(0, 2, layer, 0)

    out_cp = []
    for j in range(5):
        n = min(128, D - 128 * j)
        rs = slice(128 * j, 128 * j + n)
        for c in range(8):
            lo = xres[rs, 128 * c:128 * c + 128].astype(jnp.bfloat16).astype(jnp.float32)
            hi = xres[rs, 1024 + 128 * c:1024 + 128 * c + 128].astype(jnp.bfloat16).astype(jnp.float32)
            wd = (pltpu.bitcast(lo, U32) >> 16) | pltpu.bitcast(hi, U32)
            if n < 128:
                wd = jnp.concatenate([wd, jnp.zeros((128 - n, 128), U32)], axis=0)
            pscr[j, pl.ds(c, 128, stride=8), :] = wd.T
        xt = pltpu.bitcast(pscr[j], jnp.bfloat16).T
        xin[rs, :] = xt[0:n, :]
        cp = pltpu.make_async_copy(xin.at[rs], o_hbm.at[rs], sems.at[j])
        cp.start()
        out_cp.append(cp)
    for cp in out_cp:
        cp.wait()


@jax.jit
def pallas_interleave_layers__sliding_local_dilated__glu_gated_geglu__prompt_kernel(
        A_x, A_wqkv, A_wo, B_x, B_w_gate, B_w_up, B_w_down):
    xT = A_x.reshape(S, D).T
    wdT = B_w_down.T
    hbm = pl.BlockSpec(memory_space=pltpu.HBM)
    bf = jnp.bfloat16
    outT = pl.pallas_call(
        _kernel,
        out_shape=jax.ShapeDtypeStruct((D, S), bf),
        in_specs=[hbm] * 6,
        out_specs=hbm,
        scratch_shapes=[
            pltpu.VMEM((D, S), bf),
            pltpu.VMEM((D, 3 * D), bf),
            pltpu.VMEM((D, D), bf),
            pltpu.VMEM((7, 384, F), bf),
            pltpu.VMEM((7, 288, F // 2), bf),
            pltpu.VMEM((3 * D, D), bf),
            pltpu.VMEM((D, D), bf),
            pltpu.VMEM((D, D), bf),
            pltpu.VMEM((D, S), jnp.float32),
            pltpu.VMEM((8, D, 128), jnp.float32),
            pltpu.VMEM((15, D, 128), jnp.float32),
            pltpu.VMEM((15, D, 128), jnp.float32),
            pltpu.VMEM((D, 1024), jnp.float32),
            pltpu.VMEM((5, 1024, 128), U32),
            pltpu.VMEM((7, T2, 384), bf),
            pltpu.SemaphoreType.DMA((8,)),
        ],
        compiler_params=pltpu.CompilerParams(vmem_limit_bytes=100 * 1024 * 1024),
    )(xT, A_wqkv, A_wo, B_w_gate, B_w_up, wdT)
    return outT.T.reshape(1, S, D)
```
